```python
import os as _os
_os.environ.setdefault("JAX_PLATFORMS", "cpu")
import jax
import jax.numpy as jnp

def _softmax(x, axis=-1):
    return jax.nn.softmax(x, axis=axis)
def _gelu(x):
    return jax.nn.gelu(x, approximate=True)
def _silu(x):
    return jax.nn.silu(x)
def _sigmoid(x):
    return jax.nn.sigmoid(x)
def _layernorm(x, axis=-1, eps=1e-5):
    m = jnp.mean(x, axis=axis, keepdims=True)
    v = jnp.var(x, axis=axis, keepdims=True)
    return (x - m) / jnp.sqrt(v + eps)
def _scatter_add(tgt, idx, src, axis=0):
    return tgt.at[idx].add(src)
def _segment_sum(src, seg, n):
    return jax.ops.segment_sum(src, seg, n)
class _Rng:
    def __init__(self, key):
        self._k = key
    def _next(self):
        self._k, sub = jax.random.split(self._k)
        return sub
    def normal(self, shape):
        return jax.random.normal(self._next(), shape, dtype=jnp.bfloat16)
    def randint(self, lo, hi, shape):
        return jax.random.randint(self._next(), shape, lo, hi, dtype=jnp.int32)
    def uniform(self, shape, lo=0.0, hi=1.0):
        return jax.random.uniform(self._next(), shape, jnp.bfloat16, lo, hi)
    def permutation(self, n):
        return jax.random.permutation(self._next(), n)


kernel_name = 'standalone__mha_softmax__near_ridge'

def setup_inputs():
    _rng = _Rng(jax.random.key(int.from_bytes(__import__("os").urandom(4), "little")))
    _w = (lambda a: (lambda t: t.astype(jnp.bfloat16) if jnp.issubdtype(t.dtype, jnp.floating) else t)(jnp.asarray(a)))
    B, H, Sq, Sk, D = 8, 32, 384, 512, 128
    return {
        "q": _w((lambda *s: _rng.normal(s) * 0.4)(B, H, Sq, D)),
        "k": _w((lambda *s: _rng.normal(s) * 0.4)(B, H, Sk, D)),
        "v": _w((lambda *s: _rng.normal(s) * 0.05)(B, H, Sk, D)),
    }

def reference(q, k, v):
    scale = q.shape[-1] ** -0.5
    scores = jnp.einsum("bhqd,bhkd->bhqk", q, k) * scale
    p = _softmax(scores, axis=-1)
    return jnp.einsum("bhqk,bhkd->bhqd", p, v)
```

```python
import functools

import jax
import jax.numpy as jnp
import jax.experimental.pallas as pl
import jax.experimental.pallas.tpu as pltpu

_NT = (((1,), (1,)), ((), ()))
_NN = (((1,), (0,)), ((), ()))


def _attn_kernel(q_ref, k_ref, v_ref, o_ref, *, hb, scale):
    for h in range(hb):
        q = q_ref[h]
        k = k_ref[h]
        v = v_ref[h]
        s = jax.lax.dot_general(q, k, _NT, preferred_element_type=jnp.float32)
        m = jnp.max(s, axis=-1, keepdims=True)
        p = jnp.exp((s - m) * scale)
        l = jnp.sum(p, axis=-1, keepdims=True)
        o = jax.lax.dot_general(p.astype(jnp.bfloat16), v, _NN,
                                preferred_element_type=jnp.float32)
        o_ref[h] = (o / l).astype(o_ref.dtype)


@jax.jit
def pallas_standalone__mha_softmax__near_ridge_kernel(
    q: jax.Array,
    k: jax.Array,
    v: jax.Array,
):
    B, H, Sq, D = q.shape
    Sk = k.shape[2]
    BH = B * H
    hb = 4
    scale = float(D) ** -0.5
    q3 = q.reshape(BH, Sq, D)
    k3 = k.reshape(BH, Sk, D)
    v3 = v.reshape(BH, Sk, D)
    out = pl.pallas_call(
        functools.partial(_attn_kernel, hb=hb, scale=scale),
        grid=(BH // hb,),
        in_specs=[
            pl.BlockSpec((hb, Sq, D), lambda i: (i, 0, 0)),
            pl.BlockSpec((hb, Sk, D), lambda i: (i, 0, 0)),
            pl.BlockSpec((hb, Sk, D), lambda i: (i, 0, 0)),
        ],
        out_specs=pl.BlockSpec((hb, Sq, D), lambda i: (i, 0, 0)),
        out_shape=jax.ShapeDtypeStruct((BH, Sq, D), q.dtype),
        compiler_params=pltpu.CompilerParams(
            dimension_semantics=("parallel",),
            vmem_limit_bytes=64 * 1024 * 1024,
        ),
    )(q3, k3, v3)
    return out.reshape(B, H, Sq, D)
```

```python
import functools

import jax
import jax.numpy as jnp
import jax.experimental.pallas as pl
import jax.experimental.pallas.tpu as pltpu

_NT = (((1,), (1,)), ((), ()))
_NN = (((1,), (0,)), ((), ()))
_LOG2E = 1.4426950408889634

_HB = 4
_RING = 17
_TAIL = 13
_WROWS = 16


def _write_schedule(nsteps, hb):
    jw = nsteps - _TAIL
    done = jw * hb
    sched = {}
    step, h0 = jw, 0
    while done - h0 >= 128:
        sched[step] = [(h0, 64)]
        step, h0 = step + 1, h0 + 64
    sched[step] = [(h0, done - h0)]
    late = nsteps - 4
    sched[late] = [(done, late * hb - done)]
    sched[nsteps] = [(late * hb, (nsteps - late) * hb)]
    return jw, sched


def _attn_kernel(q_hbm, k_hbm, v_hbm, o_hbm, qb, kb, vb, ob, isem, osem, *,
                 hb, ring, nsteps, jw, sched, exp2_scale):
    i = pl.program_id(0)
    sq = ob.shape[1]

    def in_copies(step):
        slot = step % ring
        heads = pl.ds(step * hb, hb)
        return [
            pltpu.make_async_copy(q_hbm.at[heads], qb.at[slot], isem.at[0, slot]),
            pltpu.make_async_copy(k_hbm.at[heads], kb.at[slot], isem.at[1, slot]),
            pltpu.make_async_copy(v_hbm.at[heads], vb.at[slot], isem.at[2, slot]),
        ]

    def flush(groups):
        for h0, n in groups:
            for r0 in range(0, sq, _WROWS):
                blk = (pl.ds(h0, n), pl.ds(r0, _WROWS))
                pltpu.make_async_copy(ob.at[blk], o_hbm.at[blk], osem).start()

    @pl.when(i == 0)
    def _():
        for s in range(ring - 1):
            for c in in_copies(s):
                c.start()

    @pl.when(i + ring - 1 < nsteps)
    def _():
        for c in in_copies(i + ring - 1):
            c.start()

    @pl.when(jnp.logical_or(i <= jw, i == nsteps - 1))
    def _():
        for c in in_copies(i):
            c.wait()

    @pl.when(i == jw)
    def _():
        for s in range(jw + 1, nsteps - 1):
            for c in in_copies(s):
                c.wait()

    for st, groups in sched.items():
        if st < nsteps:
            pl.when(i == st)(functools.partial(flush, groups))

    slot = i % ring
    for h in range(hb):
        q = qb[slot, h]
        k = kb[slot, h]
        v = vb[slot, h]
        s = jax.lax.dot_general(q, k, _NT, preferred_element_type=jnp.float32)
        m = jnp.max(s, axis=-1, keepdims=True)
        p = jnp.exp2((s - m) * exp2_scale)
        l = jnp.sum(p, axis=-1, keepdims=True)
        o = jax.lax.dot_general(p.astype(v.dtype), v, _NN,
                                preferred_element_type=jnp.float32)
        ob[i * hb + h] = (o * pl.reciprocal(l, approx=True)).astype(ob.dtype)

    @pl.when(i == nsteps - 1)
    def _():
        flush(sched[nsteps])
        pltpu.make_async_copy(ob, o_hbm, osem).wait()


@jax.jit
def pallas_standalone__mha_softmax__near_ridge_kernel(
    q: jax.Array,
    k: jax.Array,
    v: jax.Array,
):
    B, H, Sq, D = q.shape
    Sk = k.shape[2]
    BH = B * H
    hb, ring = _HB, _RING
    assert BH % hb == 0 and Sq % _WROWS == 0
    nsteps = BH // hb
    jw, sched = _write_schedule(nsteps, hb)
    assert jw + ring - 1 >= nsteps
    exp2_scale = float(D) ** -0.5 * _LOG2E

    out = pl.pallas_call(
        functools.partial(_attn_kernel, hb=hb, ring=ring, nsteps=nsteps, jw=jw,
                          sched=sched, exp2_scale=exp2_scale),
        grid=(nsteps,),
        in_specs=[pl.BlockSpec(memory_space=pl.ANY)] * 3,
        out_specs=pl.BlockSpec(memory_space=pl.ANY),
        out_shape=jax.ShapeDtypeStruct((BH, Sq, D), q.dtype),
        scratch_shapes=[
            pltpu.VMEM((ring, hb, Sq, D), q.dtype),
            pltpu.VMEM((ring, hb, Sk, D), k.dtype),
            pltpu.VMEM((ring, hb, Sk, D), v.dtype),
            pltpu.VMEM((BH, Sq, D), q.dtype),
            pltpu.SemaphoreType.DMA((3, ring)),
            pltpu.SemaphoreType.DMA(()),
        ],
        compiler_params=pltpu.CompilerParams(
            dimension_semantics=("arbitrary",),
            vmem_limit_bytes=100 * 1024 * 1024,
        ),
    )(q.reshape(BH, Sq, D), k.reshape(BH, Sk, D), v.reshape(BH, Sk, D))
    return out.reshape(B, H, Sq, D)
```

```python
import functools

import jax
import jax.numpy as jnp
import jax.experimental.pallas as pl
import jax.experimental.pallas.tpu as pltpu

_NT = (((1,), (1,)), ((), ()))
_NN = (((1,), (0,)), ((), ()))
_LOG2E = 1.4426950408889634

_HS = 8
_CH = _HS // 2
_RING = 36
_PIECES = 4
_AROWS = 16
_WROWS = 16
_WGROUP = 64


def _plan(nsteps):
    per_ring = nsteps * _CH
    n_init = 2 * _CH
    skip = 5
    n_issue = next(s for s in range(1, nsteps)
                   if n_init + 5 * s - s // skip >= per_ring)
    assert n_init + 5 * n_issue - n_issue // skip == per_ring
    for s in range(n_issue):
        last = n_init + 5 * s - s // skip + (3 if s % skip == skip - 1 else 4)
        assert last - _RING < _CH * s and last < per_ring
    done = n_issue * _HS
    flush, step, h0 = {}, n_issue, 0
    while done - h0 >= 2 * _WGROUP:
        flush[step] = [(h0, _WGROUP)]
        step, h0 = step + 1, h0 + _WGROUP
    flush[step] = [(h0, done - h0)]
    late = nsteps - 2
    assert step < late
    flush[late] = [(done, late * _HS - done)]
    flush[nsteps] = [(late * _HS, (nsteps - late) * _HS)]
    return n_init, n_issue, skip, flush


def _head_events(sq, sk):
    qr, kr = sq // _PIECES, sk // _PIECES
    return [[(0, j * qr, qr, 0), (1, j * kr, kr, 1), (2, j * kr, kr, 1)]
            for j in range(_PIECES)]


def _anchor_plan(events):
    reg = [(hh, ev) for hh in range(_CH) for ev in events]
    seq, k = [], 0
    for t, x in enumerate(reg):
        seq.append(x)
        if (t + 1) * len(events) // len(reg) > k:
            seq.append((_CH, events[k]))
            k += 1
    n = _CH * _PIECES
    plan = [[] for _ in range(n)]
    for t, (hh, ev) in enumerate(seq):
        plan[t * n // len(seq)] += [(hh, pc) for pc in ev]
    return plan


def _attn_kernel(q_hbm, k_hbm, v_hbm, o_hbm, z0, z1, ob, sink, isem, osem, ksem,
                 *, nsteps, n_init, n_issue, skip, flush_at, exp2_scale):
    i = pl.program_id(0)
    rings = (z0, z1)
    srcs = (q_hbm, k_hbm, v_hbm)
    sq, sk = q_hbm.shape[2], k_hbm.shape[2]
    offs = (0, sq, sq + sk)
    per_ring = nsteps * _CH
    nchunks = _RING // _CH
    events = _head_events(sq, sk)
    plan = _anchor_plan(events)

    def fetch(e, n, piece):
        a, r0, nr, prio = piece
        sem = jnp.where(n == per_ring - 1, nchunks, (n // _CH) % nchunks)
        pltpu.make_async_copy(
            srcs[a].at[n, e, pl.ds(r0, nr)],
            rings[e].at[n % _RING, pl.ds(offs[a] + r0, nr)],
            isem.at[e, sem]).start(priority=prio)

    def wait_heads(e, slot, count, sem):
        sl = rings[e].at[pl.ds(slot, count)]
        pltpu.make_async_copy(sl, sl, isem.at[e, sem]).wait()

    def wait_chunk(ch, count=_CH):
        for e in range(2):
            wait_heads(e, (ch % nchunks) * _CH, count, ch % nchunks)

    def flush(groups):
        for h0, n in groups:
            for r0 in range(0, sq, _WROWS):
                blk = (pl.ds(h0, n), pl.ds(r0, _WROWS))
                pltpu.make_async_copy(ob.at[blk], o_hbm.at[blk], osem).start()

    @pl.when(i == 0)
    def _():
        for n in range(n_init):
            for e in range(2):
                for ev in events:
                    for piece in ev:
                        fetch(e, n, piece)

    @pl.when(i <= n_issue)
    def _():
        wait_chunk(i)

    @pl.when(i == n_issue)
    def _():
        for ch in range(n_issue + 1, nsteps):
            wait_chunk(ch, _CH - 1 if ch == nsteps - 1 else _CH)

    @pl.when(i == n_issue + 1)
    def _():
        for e in range(2):
            wait_heads(e, (per_ring - 1) % _RING, 1, nchunks)

    for st, groups in flush_at.items():
        if st < nsteps:
            pl.when(i == st)(functools.partial(flush, groups))

    n0 = n_init + 5 * i - i // skip
    issue = i < n_issue
    issue5 = jnp.logical_and(issue, i % skip != skip - 1)
    slot0 = (i % nchunks) * _CH

    def scores(h):
        e = h % 2
        z = rings[e]
        q = z[slot0 + h // 2, 0:sq]
        k = z[slot0 + h // 2, sq:sq + sk]
        s = jax.lax.dot_general(q, k, _NT, preferred_element_type=jnp.float32)
        m = jnp.max(s, axis=-1, keepdims=True)
        p = jnp.exp2((s - m) * exp2_scale)
        l = jnp.sum(p, axis=-1, keepdims=True)
        for t in range(_PIECES):
            a = (h // 2) * _PIECES + t
            r1 = (t + 1) * (sq // _PIECES)
            z[_RING, a * _AROWS:(a + 1) * _AROWS, :] = (
                p[r1 - _AROWS:r1, 0:z.shape[2]].astype(z.dtype))
            for hh, piece in plan[a]:
                n = jnp.minimum(n0 + hh, per_ring - 1)
                pl.when(issue5 if hh == _CH else issue)(
                    functools.partial(fetch, e, n, piece))
        return p.astype(z.dtype), l

    def output(h, p, l):
        v = rings[h % 2][slot0 + h // 2, sq + sk:sq + 2 * sk]
        o = jax.lax.dot_general(p, v, _NN, preferred_element_type=jnp.float32)
        ob[i * _HS + h] = (o * pl.reciprocal(l, approx=True)).astype(ob.dtype)

    cur = scores(0)
    for h in range(_HS):
        nxt = scores(h + 1) if h + 1 < _HS else None
        output(h, *cur)
        cur = nxt

    @pl.when(i == nsteps - 1)
    def _():
        flush(flush_at[nsteps])
        for e in range(2):
            cp = pltpu.make_async_copy(
                rings[e].at[_RING, pl.ds(0, sink.shape[0])], sink, ksem)
            cp.start()
            cp.wait()
        pltpu.make_async_copy(ob, o_hbm, osem).wait()


@jax.jit
def pallas_standalone__mha_softmax__near_ridge_kernel(
    q: jax.Array,
    k: jax.Array,
    v: jax.Array,
):
    B, H, Sq, D = q.shape
    Sk = k.shape[2]
    BH = B * H
    assert BH % _HS == 0 and D == 128
    assert Sq % (16 * _PIECES) == 0 and Sk % (16 * _PIECES) == 0
    nsteps = BH // _HS
    n_init, n_issue, skip, flush_at = _plan(nsteps)
    slot_rows = Sq + 2 * Sk

    out = pl.pallas_call(
        functools.partial(
            _attn_kernel, nsteps=nsteps, n_init=n_init, n_issue=n_issue,
            skip=skip, flush_at=flush_at,
            exp2_scale=float(D) ** -0.5 * _LOG2E),
        grid=(nsteps,),
        in_specs=[pl.BlockSpec(memory_space=pl.ANY)] * 3,
        out_specs=pl.BlockSpec(memory_space=pl.ANY),
        out_shape=jax.ShapeDtypeStruct((BH, Sq, D), q.dtype),
        scratch_shapes=[
            pltpu.VMEM((_RING + 1, slot_rows, D), q.dtype),
            pltpu.VMEM((_RING + 1, slot_rows, D), q.dtype),
            pltpu.VMEM((BH, Sq, D), q.dtype),
            pltpu.VMEM((_CH * _PIECES * _AROWS, D), q.dtype),
            pltpu.SemaphoreType.DMA((2, _RING // _CH + 1)),
            pltpu.SemaphoreType.DMA(()),
            pltpu.SemaphoreType.DMA(()),
        ],
        compiler_params=pltpu.CompilerParams(
            dimension_semantics=("arbitrary",),
            vmem_limit_bytes=100 * 1024 * 1024,
            disable_bounds_checks=True,
        ),
    )(q.reshape(BH // 2, 2, Sq, D), k.reshape(BH // 2, 2, Sk, D),
      v.reshape(BH // 2, 2, Sk, D))
    return out.reshape(B, H, Sq, D)
```

```python
import functools

import jax
import jax.numpy as jnp
import jax.experimental.pallas as pl
import jax.experimental.pallas.tpu as pltpu

_NT = (((1,), (1,)), ((), ()))
_NN = (((1,), (0,)), ((), ()))
_LOG2E = 1.4426950408889634

_HS = 8
_CH = _HS // 2
_RING = 36
_PIECES = 4
_AROWS = 16
_WROWS = 16
_WGROUP = 64


def _plan(nsteps):
    per_ring = nsteps * _CH
    n_init = 2 * _CH
    skip = 5
    n_issue = next(s for s in range(1, nsteps)
                   if n_init + 5 * s - s // skip >= per_ring)
    assert n_init + 5 * n_issue - n_issue // skip == per_ring
    for s in range(n_issue):
        last = n_init + 5 * s - s // skip + (3 if s % skip == skip - 1 else 4)
        assert last - _RING < _CH * s and last < per_ring
    done = n_issue * _HS
    flush, step, h0 = {}, n_issue, 0
    while done - h0 >= 2 * _WGROUP:
        flush[step] = [(h0, _WGROUP)]
        step, h0 = step + 1, h0 + _WGROUP
    flush[step] = [(h0, done - h0)]
    late = nsteps - 2
    assert step < late
    flush[late] = [(done, late * _HS - done)]
    flush[nsteps] = [(late * _HS, (nsteps - late) * _HS)]
    return n_init, n_issue, skip, flush


def _head_events(sq, sk):
    qr, kr = sq // _PIECES, sk // _PIECES
    return [[(0, j * qr, qr, 0), (1, j * kr, kr, 1), (2, j * kr, kr, 1)]
            for j in range(_PIECES)]


def _anchor_plan(events):
    reg = [(hh, ev) for hh in range(_CH) for ev in events]
    seq, k = [], 0
    for t, x in enumerate(reg):
        seq.append(x)
        if (t + 1) * len(events) // len(reg) > k:
            seq.append((_CH, events[k]))
            k += 1
    n = _CH * _PIECES
    plan = [[] for _ in range(n)]
    for t, (hh, ev) in enumerate(seq):
        plan[t * n // len(seq)] += [(hh, pc) for pc in ev]
    return plan


def _attn_kernel(q_hbm, k_hbm, v_hbm, o_hbm, z0, z1, ob, sink, isem, osem, ksem,
                 *, nsteps, n_init, n_issue, skip, flush_at, exp2_scale):
    i = pl.program_id(0)
    rings = (z0, z1)
    srcs = (q_hbm, k_hbm, v_hbm)
    sq, sk = q_hbm.shape[2], k_hbm.shape[2]
    offs = (0, sq, sq + sk)
    per_ring = nsteps * _CH
    nchunks = _RING // _CH
    events = _head_events(sq, sk)
    plan = _anchor_plan(events)

    def fetch(e, n, piece):
        a, r0, nr, prio = piece
        sem = jnp.where(n == per_ring - 1, nchunks, (n // _CH) % nchunks)
        pltpu.make_async_copy(
            srcs[a].at[n, e, pl.ds(r0, nr)],
            rings[e].at[n % _RING, pl.ds(offs[a] + r0, nr)],
            isem.at[e, sem]).start(priority=prio)

    def wait_heads(e, slot, count, sem):
        sl = rings[e].at[pl.ds(slot, count)]
        pltpu.make_async_copy(sl, sl, isem.at[e, sem]).wait()

    def wait_chunk(ch, count=_CH):
        for e in range(2):
            wait_heads(e, (ch % nchunks) * _CH, count, ch % nchunks)

    def flush(groups):
        for h0, n in groups:
            for r0 in range(0, sq, _WROWS):
                blk = (pl.ds(h0, n), pl.ds(r0, _WROWS))
                pltpu.make_async_copy(ob.at[blk], o_hbm.at[blk], osem).start()

    @pl.when(i == 0)
    def _():
        for n in range(n_init):
            for e in range(2):
                for ev in events:
                    for piece in ev:
                        fetch(e, n, piece)

    @pl.when(i <= n_issue)
    def _():
        wait_chunk(i)

    @pl.when(i == n_issue)
    def _():
        for e in range(2):
            pltpu.make_async_copy(rings[e].at[_RING, pl.ds(0, sink.shape[1])],
                                  sink.at[e], ksem).start()
        for ch in range(n_issue + 1, nsteps):
            wait_chunk(ch, _CH - 1 if ch == nsteps - 1 else _CH)
        pltpu.make_async_copy(sink, sink, ksem).wait()

    @pl.when(i == n_issue + 1)
    def _():
        for e in range(2):
            wait_heads(e, (per_ring - 1) % _RING, 1, nchunks)

    for st, groups in flush_at.items():
        if st < nsteps:
            pl.when(i == st)(functools.partial(flush, groups))

    n0 = n_init + 5 * i - i // skip
    issue = i < n_issue
    issue5 = jnp.logical_and(issue, i % skip != skip - 1)
    slot0 = (i % nchunks) * _CH

    def scores(h):
        e = h % 2
        z = rings[e]
        q = z[slot0 + h // 2, 0:sq]
        k = z[slot0 + h // 2, sq:sq + sk]
        s = jax.lax.dot_general(q, k, _NT, preferred_element_type=jnp.float32)
        m = jnp.max(s, axis=-1, keepdims=True)
        p = jnp.exp2((s - m) * exp2_scale)
        l = jnp.sum(p, axis=-1, keepdims=True)
        for t in range(_PIECES):
            a = (h // 2) * _PIECES + t
            r1 = (t + 1) * (sq // _PIECES)
            z[_RING, a * _AROWS:(a + 1) * _AROWS, :] = (
                p[r1 - _AROWS:r1, 0:z.shape[2]].astype(z.dtype))
            for hh, piece in plan[a]:
                n = jnp.minimum(n0 + hh, per_ring - 1)
                pl.when(issue5 if hh == _CH else issue)(
                    functools.partial(fetch, e, n, piece))
        return p.astype(z.dtype), l

    def output(h, p, l):
        v = rings[h % 2][slot0 + h // 2, sq + sk:sq + 2 * sk]
        o = jax.lax.dot_general(p, v, _NN, preferred_element_type=jnp.float32)
        ob[i * _HS + h] = (o * pl.reciprocal(l, approx=True)).astype(ob.dtype)

    cur = scores(0)
    for h in range(_HS):
        nxt = scores(h + 1) if h + 1 < _HS else None
        output(h, *cur)
        cur = nxt

    @pl.when(i == nsteps - 1)
    def _():
        flush(flush_at[nsteps])
        pltpu.make_async_copy(ob, o_hbm, osem).wait()


@jax.jit
def pallas_standalone__mha_softmax__near_ridge_kernel(
    q: jax.Array,
    k: jax.Array,
    v: jax.Array,
):
    B, H, Sq, D = q.shape
    Sk = k.shape[2]
    BH = B * H
    assert BH % _HS == 0 and D == 128
    assert Sq % (16 * _PIECES) == 0 and Sk % (16 * _PIECES) == 0
    nsteps = BH // _HS
    n_init, n_issue, skip, flush_at = _plan(nsteps)
    slot_rows = Sq + 2 * Sk

    out = pl.pallas_call(
        functools.partial(
            _attn_kernel, nsteps=nsteps, n_init=n_init, n_issue=n_issue,
            skip=skip, flush_at=flush_at,
            exp2_scale=float(D) ** -0.5 * _LOG2E),
        grid=(nsteps,),
        in_specs=[pl.BlockSpec(memory_space=pl.ANY)] * 3,
        out_specs=pl.BlockSpec(memory_space=pl.ANY),
        out_shape=jax.ShapeDtypeStruct((BH, Sq, D), q.dtype),
        scratch_shapes=[
            pltpu.VMEM((_RING + 1, slot_rows, D), q.dtype),
            pltpu.VMEM((_RING + 1, slot_rows, D), q.dtype),
            pltpu.VMEM((BH, Sq, D), q.dtype),
            pltpu.VMEM((2, _CH * _PIECES * _AROWS, D), q.dtype),
            pltpu.SemaphoreType.DMA((2, _RING // _CH + 1)),
            pltpu.SemaphoreType.DMA(()),
            pltpu.SemaphoreType.DMA(()),
        ],
        compiler_params=pltpu.CompilerParams(
            dimension_semantics=("arbitrary",),
            vmem_limit_bytes=100 * 1024 * 1024,
            disable_bounds_checks=True,
        ),
    )(q.reshape(BH // 2, 2, Sq, D), k.reshape(BH // 2, 2, Sk, D),
      v.reshape(BH // 2, 2, Sk, D))
    return out.reshape(B, H, Sq, D)
```

```python
import functools

import jax
import jax.numpy as jnp
import jax.experimental.pallas as pl
import jax.experimental.pallas.tpu as pltpu

_NT = (((1,), (1,)), ((), ()))
_NN = (((1,), (0,)), ((), ()))
_LOG2E = 1.4426950408889634

_HS = 8
_CH = _HS // 2
_RING = 36
_PIECES = 4
_AROWS = 16
_WROWS = 16
_WGROUP = 64


def _plan(nsteps):
    per_ring = nsteps * _CH
    n_init = 2 * _CH
    skip = 5
    n_issue = next(s for s in range(1, nsteps)
                   if n_init + 5 * s - s // skip >= per_ring)
    assert n_init + 5 * n_issue - n_issue // skip == per_ring
    for s in range(n_issue):
        last = n_init + 5 * s - s // skip + (3 if s % skip == skip - 1 else 4)
        assert last - _RING < _CH * s and last < per_ring
    done = n_issue * _HS
    flush, step, h0 = {}, n_issue, 0
    while done - h0 >= _WGROUP:
        flush[step] = [(h0, _WGROUP)]
        step, h0 = step + 1, h0 + _WGROUP
    late = nsteps - 2
    assert step <= late
    flush[late] = [(h0, late * _HS - h0)]
    flush[nsteps] = [(late * _HS, (nsteps - late) * _HS)]
    assert all(h + n <= st * _HS for st, g in flush.items() for h, n in g)
    assert sum(n for g in flush.values() for _, n in g) == nsteps * _HS
    return n_init, n_issue, skip, flush


def _head_events(sq, sk):
    qr, kr = sq // _PIECES, sk // _PIECES
    return [[(0, j * qr, qr, 0), (1, j * kr, kr, 1), (2, j * kr, kr, 1)]
            for j in range(_PIECES)]


def _anchor_plan(events):
    reg = [(hh, ev) for hh in range(_CH) for ev in events]
    seq, k = [], 0
    for t, x in enumerate(reg):
        seq.append(x)
        if (t + 1) * len(events) // len(reg) > k:
            seq.append((_CH, events[k]))
            k += 1
    n = _CH * _PIECES
    plan = [[] for _ in range(n)]
    for t, (hh, ev) in enumerate(seq):
        plan[t * n // len(seq)] += [(hh, pc) for pc in ev]
    return plan


def _attn_kernel(q_hbm, k_hbm, v_hbm, o_hbm, z0, z1, ob, sink, isem, osem, ksem,
                 *, nsteps, n_init, n_issue, skip, flush_at, exp2_scale):
    i = pl.program_id(0)
    rings = (z0, z1)
    srcs = (q_hbm, k_hbm, v_hbm)
    sq, sk = q_hbm.shape[2], k_hbm.shape[2]
    offs = (0, sq, sq + sk)
    per_ring = nsteps * _CH
    nchunks = _RING // _CH
    events = _head_events(sq, sk)
    plan = _anchor_plan(events)

    def fetch(e, n, piece):
        a, r0, nr, prio = piece
        sem = jnp.where(n == per_ring - 1, nchunks, (n // _CH) % nchunks)
        pltpu.make_async_copy(
            srcs[a].at[n, e, pl.ds(r0, nr)],
            rings[e].at[n % _RING, pl.ds(offs[a] + r0, nr)],
            isem.at[e, sem]).start(priority=prio)

    def wait_heads(e, slot, count, sem):
        sl = rings[e].at[pl.ds(slot, count)]
        pltpu.make_async_copy(sl, sl, isem.at[e, sem]).wait()

    def wait_chunk(ch, count=_CH):
        for e in range(2):
            wait_heads(e, (ch % nchunks) * _CH, count, ch % nchunks)

    def flush(groups):
        for h0, n in groups:
            for r0 in range(0, sq, _WROWS):
                blk = (pl.ds(h0, n), pl.ds(r0, _WROWS))
                pltpu.make_async_copy(ob.at[blk], o_hbm.at[blk], osem).start()

    @pl.when(i == 0)
    def _():
        for n in range(n_init):
            for e in range(2):
                for ev in events:
                    for piece in ev:
                        fetch(e, n, piece)

    @pl.when(i <= n_issue)
    def _():
        wait_chunk(i)

    @pl.when(i == n_issue)
    def _():
        for e in range(2):
            pltpu.make_async_copy(rings[e].at[_RING, pl.ds(0, sink.shape[1])],
                                  sink.at[e], ksem).start()
        for ch in range(n_issue + 1, nsteps):
            wait_chunk(ch, _CH - 1 if ch == nsteps - 1 else _CH)
        pltpu.make_async_copy(sink, sink, ksem).wait()

    @pl.when(i == n_issue + 1)
    def _():
        for e in range(2):
            wait_heads(e, (per_ring - 1) % _RING, 1, nchunks)

    for st, groups in flush_at.items():
        if st < nsteps:
            pl.when(i == st)(functools.partial(flush, groups))

    n0 = n_init + 5 * i - i // skip
    issue = i < n_issue
    issue5 = jnp.logical_and(issue, i % skip != skip - 1)
    slot0 = (i % nchunks) * _CH

    def scores(h):
        e = h % 2
        z = rings[e]
        q = z[slot0 + h // 2, 0:sq]
        k = z[slot0 + h // 2, sq:sq + sk]
        s = jax.lax.dot_general(q, k, _NT, preferred_element_type=jnp.float32)
        m = jnp.max(s, axis=-1, keepdims=True)
        p = jnp.exp2((s - m) * exp2_scale)
        l = jnp.sum(p, axis=-1, keepdims=True)
        for t in range(_PIECES):
            a = (h // 2) * _PIECES + t
            r1 = (t + 1) * (sq // _PIECES)
            z[_RING, a * _AROWS:(a + 1) * _AROWS, :] = (
                p[r1 - _AROWS:r1, 0:z.shape[2]].astype(z.dtype))
            for hh, piece in plan[a]:
                n = jnp.minimum(n0 + hh, per_ring - 1)
                pl.when(issue5 if hh == _CH else issue)(
                    functools.partial(fetch, e, n, piece))
        return p.astype(z.dtype), l

    def output(h, p, l):
        v = rings[h % 2][slot0 + h // 2, sq + sk:sq + 2 * sk]
        o = jax.lax.dot_general(p, v, _NN, preferred_element_type=jnp.float32)
        ob[i * _HS + h] = (o * pl.reciprocal(l, approx=True)).astype(ob.dtype)

    cur = scores(0)
    for h in range(_HS):
        nxt = scores(h + 1) if h + 1 < _HS else None
        output(h, *cur)
        cur = nxt

    @pl.when(i == nsteps - 1)
    def _():
        flush(flush_at[nsteps])
        pltpu.make_async_copy(ob, o_hbm, osem).wait()


@jax.jit
def pallas_standalone__mha_softmax__near_ridge_kernel(
    q: jax.Array,
    k: jax.Array,
    v: jax.Array,
):
    B, H, Sq, D = q.shape
    Sk = k.shape[2]
    BH = B * H
    assert BH % _HS == 0 and D == 128
    assert Sq % (16 * _PIECES) == 0 and Sk % (16 * _PIECES) == 0
    nsteps = BH // _HS
    n_init, n_issue, skip, flush_at = _plan(nsteps)
    slot_rows = Sq + 2 * Sk

    out = pl.pallas_call(
        functools.partial(
            _attn_kernel, nsteps=nsteps, n_init=n_init, n_issue=n_issue,
            skip=skip, flush_at=flush_at,
            exp2_scale=float(D) ** -0.5 * _LOG2E),
        grid=(nsteps,),
        in_specs=[pl.BlockSpec(memory_space=pl.ANY)] * 3,
        out_specs=pl.BlockSpec(memory_space=pl.ANY),
        out_shape=jax.ShapeDtypeStruct((BH, Sq, D), q.dtype),
        scratch_shapes=[
            pltpu.VMEM((_RING + 1, slot_rows, D), q.dtype),
            pltpu.VMEM((_RING + 1, slot_rows, D), q.dtype),
            pltpu.VMEM((BH, Sq, D), q.dtype),
            pltpu.VMEM((2, _CH * _PIECES * _AROWS, D), q.dtype),
            pltpu.SemaphoreType.DMA((2, _RING // _CH + 1)),
            pltpu.SemaphoreType.DMA(()),
            pltpu.SemaphoreType.DMA(()),
        ],
        compiler_params=pltpu.CompilerParams(
            dimension_semantics=("arbitrary",),
            vmem_limit_bytes=100 * 1024 * 1024,
            disable_bounds_checks=True,
            disable_semaphore_checks=True,
        ),
    )(q.reshape(BH // 2, 2, Sq, D), k.reshape(BH // 2, 2, Sk, D),
      v.reshape(BH // 2, 2, Sk, D))
    return out.reshape(B, H, Sq, D)
```
